```python
import os as _os
_os.environ.setdefault("JAX_PLATFORMS", "cpu")
import jax
import jax.numpy as jnp

def _softmax(x, axis=-1):
    return jax.nn.softmax(x, axis=axis)
def _gelu(x):
    return jax.nn.gelu(x, approximate=True)
def _silu(x):
    return jax.nn.silu(x)
def _sigmoid(x):
    return jax.nn.sigmoid(x)
def _layernorm(x, axis=-1, eps=1e-5):
    m = jnp.mean(x, axis=axis, keepdims=True)
    v = jnp.var(x, axis=axis, keepdims=True)
    return (x - m) / jnp.sqrt(v + eps)
def _scatter_add(tgt, idx, src, axis=0):
    return tgt.at[idx].add(src)
def _segment_sum(src, seg, n):
    return jax.ops.segment_sum(src, seg, n)
class _Rng:
    def __init__(self, key):
        self._k = key
    def _next(self):
        self._k, sub = jax.random.split(self._k)
        return sub
    def normal(self, shape):
        return jax.random.normal(self._next(), shape, dtype=jnp.bfloat16)
    def randint(self, lo, hi, shape):
        return jax.random.randint(self._next(), shape, lo, hi, dtype=jnp.int32)
    def uniform(self, shape, lo=0.0, hi=1.0):
        return jax.random.uniform(self._next(), shape, jnp.bfloat16, lo, hi)
    def permutation(self, n):
        return jax.random.permutation(self._next(), n)


kernel_name = 'concat_heads__grouped_kv_mqa__sliding_block__prompt'

def setup_inputs():
    _rng = _Rng(jax.random.key(int.from_bytes(__import__("os").urandom(4), "little")))
    _w = (lambda a: (lambda t: t.astype(jnp.bfloat16) if jnp.issubdtype(t.dtype, jnp.floating) else t)(jnp.asarray(a)))
    def _A_setup():
        B, S, D, H = 1, 2048, 576, 32
        Dh = D // H
        return {
            "x": _w((lambda *s: _rng.normal(s) * 0.05)(B, S, D)),
            "wq": _w((lambda *s: _rng.normal(s) * 1.6)(D, H * Dh)),
            "wk": _w((lambda *s: _rng.normal(s) * 1.6)(D, Dh)),
            "wv": _w((lambda *s: _rng.normal(s) * 0.1)(D, Dh)),
            "wo": _w((lambda *s: _rng.normal(s) * 0.1)(H * Dh, D)),
        }
    _A_in = _A_setup()

    def _B_setup():
        B, S, D = 1, 2048, 576
        return {
            "x": _w((lambda *s: _rng.normal(s) * 0.2)(B, S, D)),
            "wqkv": _w((lambda *s: _rng.normal(s) * 0.2)(D, 3 * D)),
            "wo": _w((lambda *s: _rng.normal(s) * 0.05)(D, D)),
        }
    _B_in = _B_setup()

    return {
        "A_x": _A_in["x"],
        "A_wq": _A_in["wq"],
        "A_wk": _A_in["wk"],
        "A_wv": _A_in["wv"],
        "A_wo": _A_in["wo"],
        "B_x": _B_in["x"],
        "B_wqkv": _B_in["wqkv"],
        "B_wo": _B_in["wo"],
    }

def reference(A_x, A_wq, A_wk, A_wv, A_wo, B_x, B_wqkv, B_wo):
    def _A_ref(x, wq, wk, wv, wo):
        B, S, D = x.shape
        H = 32
        Dh = D // H
        q = (lambda x, *d: x.transpose(*d))((x @ wq).reshape(B, S, H, Dh), 0, 2, 1, 3)
        k = x @ wk
        v = x @ wv
        scores = jnp.einsum("bhqd,bkd->bhqk", q, k) * (Dh ** -0.5)
        p = _softmax(scores, axis=-1)
        o = jnp.einsum("bhqk,bkd->bhqd", p, v)
        return (lambda x, *d: x.transpose(*d))(o, 0, 2, 1, 3).reshape(B, S, H * Dh) @ wo

    def _B_ref(x, wqkv, wo):
        B, S, D = x.shape
        H = 32; Dh = D // H; W = 256
        qkv = (lambda x, *d: x.transpose(*d))((x @ wqkv).reshape(B, S, 3, H, Dh), 2, 0, 3, 1, 4)
        q, k, v = qkv[0], qkv[1], qkv[2]
        scores = jnp.einsum("bhqd,bhkd->bhqk", q, k) * (Dh ** -0.5)
        idx = jnp.arange(S)
        mask = (idx[:, None] - idx[None, :] >= 0) & (idx[:, None] - idx[None, :] < W)
        scores = jnp.where(mask[None, None], scores, -1e9)
        p = _softmax(scores, axis=-1)
        o = jnp.einsum("bhqk,bhkd->bhqd", p, v)
        return (lambda x, *d: x.transpose(*d))(o, 0, 2, 1, 3).reshape(B, S, D) @ wo

    a = _A_ref(A_x, A_wq, A_wk, A_wv, A_wo)
    b = _B_ref(B_x, B_wqkv, B_wo)
    return jnp.concatenate([a, b], axis=-1)
```

```python
import math

import jax
import jax.numpy as jnp
import numpy as np
from jax import lax
import jax.experimental.pallas as pl
import jax.experimental.pallas.tpu as pltpu

S = 2048
D = 576
H = 32
DH = D // H
W = 256
NB = 512
CH = 128
UNROLL_A = 4
QSCALE = float(DH ** -0.5 * math.log2(math.e))
NEG = -1e30

BF = jnp.bfloat16
F32 = jnp.float32


def _dot(a, b):
    return jnp.dot(a, b, preferred_element_type=F32)


def _pad_rows(x, rows):
    return jnp.concatenate(
        [x, jnp.zeros((rows - x.shape[0], x.shape[1]), x.dtype)], axis=0)


def _kernel(xa_hbm, wq_hbm, wkt_hbm, wvt_hbm, woa_hbm, xb_hbm, wqkv_hbm, wob_hbm,
            out_hbm,
            xa, xb, wq, wkt, wvt, woa, wqkv, wob,
            wat, wbt, wot,
            qa, ka, va, s_a, oa,
            qb, kb, vb, s_b, ob,
            obuf, in_sem, out_sem):
    nblk = S // NB

    copies = [pltpu.make_async_copy(wq_hbm, wq, in_sem.at[0]),
              pltpu.make_async_copy(wkt_hbm, wkt, in_sem.at[1]),
              pltpu.make_async_copy(wvt_hbm, wvt, in_sem.at[2])]
    xa_copies = [
        pltpu.make_async_copy(xa_hbm.at[:, pl.ds(n * NB, NB)],
                              xa.at[:, pl.ds(n * NB, NB)], in_sem.at[3 + n])
        for n in range(nblk)]
    late = [pltpu.make_async_copy(xb_hbm, xb, in_sem.at[7]),
            pltpu.make_async_copy(wqkv_hbm, wqkv, in_sem.at[8]),
            pltpu.make_async_copy(woa_hbm, woa, in_sem.at[9]),
            pltpu.make_async_copy(wob_hbm, wob, in_sem.at[10])]
    for c in copies + xa_copies + late:
        c.start()

    for c in copies:
        c.wait()
    wat[0:D, :] = wq[...].T
    wat[D:D + 64, :] = jnp.concatenate(
        [_pad_rows(wkt[...].astype(F32), 32),
         _pad_rows(wvt[...].astype(F32), 32)], axis=0).astype(BF)

    for n in range(nblk):
        xa_copies[n].wait()
        cols = pl.ds(n * NB, NB)
        r = _dot(wat[0:D + 56, :], xa[:, cols])
        for h in range(H):
            q = r[h * DH:(h + 1) * DH] * QSCALE
            qa[n * H + h] = _pad_rows(q, 32).astype(BF)
        kt = _pad_rows(r[D:D + 24], 128)
        ka[cols, :] = kt.T[:, 0:32].astype(BF)
        v = r[D + 32:D + 56].astype(BF).astype(F32)
        row = lax.broadcasted_iota(jnp.int32, v.shape, 0)
        va[:, cols] = jnp.where(row == DH, 1.0, v)

    def scores_chunk(c, q, mx):
        rows = pl.ds(c * CH, CH)
        s = _dot(ka[rows, :], q)
        s_a[rows, :] = s
        mc = jnp.max(s.reshape(CH // 8, 8, NB), axis=0)
        return mc if mx is None else jnp.maximum(mx, mc)

    def unit_a(u, m):
        q = qa[jnp.minimum(u + 1, nblk * H - 1)]
        mx = None
        acc = None
        for c in range(S // CH):
            rows = pl.ds(c * CH, CH)
            p = jnp.exp2(s_a[rows, :] - m).astype(BF)
            mx = scores_chunk(c, q, mx)
            o = _dot(va[:, rows], p)
            acc = o if acc is None else acc + o
        oa[u] = acc * (1.0 / acc[DH:DH + 1])
        return jnp.max(mx, axis=0, keepdims=True)

    mx = None
    q0 = qa[0]
    for c in range(S // CH):
        mx = scores_chunk(c, q0, mx)

    def body_a(i, m):
        for j in range(UNROLL_A):
            m = unit_a(i * UNROLL_A + j, m)
        return m

    lax.fori_loop(0, nblk * H // UNROLL_A, body_a,
                  jnp.max(mx, axis=0, keepdims=True))

    for c in late:
        c.wait()
    wbt[...] = wqkv[...].T
    wot[0:D, :] = woa[...].T
    wot[D:2 * D, :] = wob[...].T

    G = H // 4
    GR = 4 * DH

    def proj_b(n, carry):
        cols = pl.ds(pl.multiple_of(n * NB, NB), NB)
        x = xb[:, cols]
        rq = _dot(wbt[0:D, :], x)
        for g in range(G):
            qb[g, :, cols] = _pad_rows(rq[g * GR:(g + 1) * GR] * QSCALE, 80).astype(BF)
        rk = _dot(wbt[D:2 * D, :], x)
        for g in range(G):
            kt = _pad_rows(rk[g * GR:(g + 1) * GR], 128)
            kb[g, cols, :] = kt.T[:, 0:80].astype(BF)
        rv = _dot(wbt[2 * D:3 * D, :], x)
        for g in range(G):
            vb[g, :, cols] = rv[g * GR:(g + 1) * GR].astype(BF).astype(F32)
        return carry

    lax.fori_loop(0, nblk, proj_b, 0)

    T = S // CH
    ki = lax.broadcasted_iota(jnp.int32, (CH, NB), 0)
    qi = lax.broadcasted_iota(jnp.int32, (CH, NB), 1) & (CH - 1)
    qrow = lax.broadcasted_iota(jnp.int32, (80, CH), 0)
    vrow = lax.broadcasted_iota(jnp.int32, (24, CH), 0)
    orow = lax.broadcasted_iota(jnp.int32, (8, CH), 0)
    ones_row = [18, 0, 0, 0]

    def group_b(g, carry):
        def blocks(t):
            return [b for b in range(3) if t - 2 + b >= 0]

        def qmat(t):
            qt = qb[g, :, pl.ds(t * CH, CH)].astype(F32)
            return jnp.concatenate(
                [jnp.where((qrow >= j * DH) & (qrow < (j + 1) * DH), qt, 0.0)
                 for j in range(4)], axis=1).astype(BF)

        def scores(t, b, q, mx):
            s = _dot(kb[g, pl.ds((t - 2 + b) * CH, CH), :], q)
            if b == 0:
                s = jnp.where(qi < ki, s, NEG)
            elif b == 2:
                s = jnp.where(qi >= ki, s, NEG)
            s_b[pl.ds(b * CH, CH), :] = s
            mc = jnp.max(s.reshape(CH // 8, 8, NB), axis=0)
            return mc if mx is None else jnp.maximum(mx, mc)

        q = qmat(0)
        mx = None
        for b in blocks(0):
            mx = scores(0, b, q, mx)
        m = jnp.max(mx, axis=0, keepdims=True)
        for t in range(T):
            q = qmat(t + 1) if t + 1 < T else None
            mx = None
            acc = [None] * 4
            for b in range(3):
                if b in blocks(t):
                    p = jnp.exp2(s_b[pl.ds(b * CH, CH), :] - m).astype(BF)
                if q is not None and b in blocks(t + 1):
                    mx = scores(t + 1, b, q, mx)
                if b in blocks(t):
                    for j in range(4):
                        v = vb[g, pl.ds(16 * j, 24), pl.ds((t - 2 + b) * CH, CH)]
                        v = jnp.where(vrow == ones_row[j], 1.0, v)
                        o = _dot(v, p[:, j * CH:(j + 1) * CH])
                        acc[j] = o if acc[j] is None else acc[j] + o
            o = [a * (1.0 / a[r:r + 1]) for a, r in zip(acc, ones_row)]
            rows = [o[0][0:16],
                    jnp.where(orow < 2, o[0][16:24], o[1][0:8]),
                    o[1][8:16],
                    jnp.where(orow < 4, o[1][16:24], o[2][0:8]),
                    o[2][8:16],
                    jnp.where(orow < 6, o[2][16:24], o[3][0:8]),
                    o[3][8:24]]
            ob[g, :, pl.ds(t * CH, CH)] = jnp.concatenate(rows, axis=0)
            if q is not None:
                m = jnp.max(mx, axis=0, keepdims=True)
        return carry

    lax.fori_loop(0, G, group_b, 0)

    out_copies = []
    for n in range(nblk):
        cols = pl.ds(n * NB, NB)
        a = jnp.concatenate([oa[n * H + h, 0:DH, :] for h in range(H)], axis=0)
        b = jnp.concatenate([ob[g, :, cols] for g in range(G)], axis=0)
        ra = _dot(wot[0:D, :], a.astype(BF))
        rb = _dot(wot[D:2 * D, :], b.astype(BF))
        obuf[n] = jnp.concatenate([ra, rb], axis=0).T.astype(BF)
        c = pltpu.make_async_copy(obuf.at[n], out_hbm.at[pl.ds(n * NB, NB), :],
                                  out_sem.at[n])
        c.start()
        out_copies.append(c)
    for c in out_copies:
        c.wait()


@jax.jit
def pallas_concat_heads__grouped_kv_mqa__sliding_block__prompt_kernel(
    A_x: jax.Array,
    A_wq: jax.Array,
    A_wk: jax.Array,
    A_wv: jax.Array,
    A_wo: jax.Array,
    B_x: jax.Array,
    B_wqkv: jax.Array,
    B_wo: jax.Array,
):
    nblk = S // NB
    hbm = pl.BlockSpec(memory_space=pltpu.HBM)
    scratch = [
        pltpu.VMEM((D, S), BF), pltpu.VMEM((D, S), BF),
        pltpu.VMEM((D, D), BF), pltpu.VMEM((DH, D), BF), pltpu.VMEM((DH, D), BF),
        pltpu.VMEM((D, D), BF), pltpu.VMEM((D, 3 * D), BF), pltpu.VMEM((D, D), BF),
        pltpu.VMEM((D + 64, D), BF), pltpu.VMEM((3 * D, D), BF),
        pltpu.VMEM((2 * D, D), BF),
        pltpu.VMEM((nblk * H, 32, NB), BF), pltpu.VMEM((S, 32), BF),
        pltpu.VMEM((24, S), F32), pltpu.VMEM((S, NB), F32),
        pltpu.VMEM((nblk * H, 24, NB), F32),
        pltpu.VMEM((H // 4, 80, S), BF), pltpu.VMEM((H // 4, S, 80), BF),
        pltpu.VMEM((H // 4, 4 * DH, S), F32), pltpu.VMEM((3 * CH, NB), F32),
        pltpu.VMEM((H // 4, 4 * DH, S), F32),
        pltpu.VMEM((nblk, NB, 2 * D), BF),
        pltpu.SemaphoreType.DMA((11,)), pltpu.SemaphoreType.DMA((nblk,)),
    ]
    out = pl.pallas_call(
        _kernel,
        in_specs=[hbm] * 8,
        out_specs=hbm,
        out_shape=jax.ShapeDtypeStruct((S, 2 * D), BF),
        scratch_shapes=scratch,
        compiler_params=pltpu.CompilerParams(vmem_limit_bytes=100 * 2**20),
        name="fused_attn",
    )(A_x[0].T, A_wq, A_wk.T, A_wv.T, A_wo, B_x[0].T, B_wqkv, B_wo)
    return out.reshape(1, S, 2 * D)
```

```python
import functools
import math

import jax
import jax.numpy as jnp
import numpy as np
from jax import lax
import jax.experimental.pallas as pl
import jax.experimental.pallas.tpu as pltpu

S = 2048
D = 576
H = 32
DH = D // H
L = 128
NT = 4
NB = NT * L
NBLK = S // NB
NCH = S // L
UNITS = NBLK * H
U = 4
NCC = U * NCH
G = H // 4
GR = 4 * DH
KROWS = S // 2 + 48
NSTEP = 15
OUT_NB = 256
ONES_ROW = (18, 0, 0, 0)
SCALE = float(DH ** -0.5 * math.log2(math.e))
NEG = -1e30
MIN_DENOM = 2.0 ** -80
MAX_DENOM = 2.0 ** 12

BF = jnp.bfloat16
F32 = jnp.float32
I32 = jnp.int32

TILE_ORDER = (2, 3, 0, 1)
VPU_SLOTS = (
    0, 1, 3, 4, 7, 10, 11, 13, 15, 17, 18, 20, 23, 25, 27, 28, 30, 32, 34, 35, 37,
    39, 41, 43, 45, 47, 48, 50, 53, 55, 57, 58, 61, 63, 64, 66, 68, 69, 72, 74, 76, 78,
    79, 82, 84, 85, 86, 87, 90, 93, 95, 96, 98, 100, 102, 104, 106, 108, 109, 112, 114,
    115, 117, 118, 121, 123, 125, 126, 128, 130, 133, 135, 137, 139, 141, 143, 145, 147,
    148, 150, 153, 155, 156, 157)
VPU_FIRST = 200


def _schedule():
    picks = [(TILE_ORDER[i % NT], x // 10, x % 10) for i, x in enumerate(VPU_SLOTS)]
    used = {(c, 7 - k) for _, c, k in picks if k < 8}
    pos = [[[] for _ in range(NT)] for _ in range(NCC)]
    tied = {}
    rest = [[] for _ in range(NT)]

    def free_group(cc, tiles):
        groups = [g for g in range(8) if all(g not in pos[cc][t] for t in tiles)]
        g = min(groups, key=lambda g: ((cc % NCH, g) not in used, g))
        used.add((cc % NCH, g))
        for t in tiles:
            pos[cc][t].append(g)
        return g

    for t, c, k in sorted(picks, key=lambda x: x[2] >= 8):
        for cc in range(c, NCC, NCH):
            if k < 8:
                pos[cc][t].append(7 - k)
                if cc == 0:
                    rest[t].append((cc, 7 - k))
            elif 0 < cc < NCC - 1:
                tied.setdefault(cc, []).append((9 - k, t, free_group(cc + 1, [t])))
            else:
                rest[t].append(((cc + 1) % NCC, free_group((cc + 1) % NCC, [t])))
    for cc in range(NCC):
        if cc % 8 == 4 or cc == 0:
            g = free_group(cc, range(NT))
            for t in range(NT):
                rest[t].append((cc, g))

    chunk, lat, work = 129, 95, 75
    skew = lambda t: 4 * ((0.0, 0.1, 0.5, 0.6)[(t + 2) % NT] + 0.6)
    slots = [(24 + lat - chunk + 8 * r + skew(t), t, "k", NCC - 2, r)
             for r in range(2, 12) for t in range(NT)]
    slots += [(24 + lat + 8 * r + skew(t), t, "k", NCC - 1, r)
              for r in range(12) for t in range(NT)]
    slots += [(chunk + k * GR + lat + 8 * r + skew(t), t, "s", k, r)
              for k in range(NSTEP) for r in range(GR // 8) for t in range(NT)]
    other = [(0, chunk, 108), (chunk, lat, 108 * lat / chunk)]
    other += [(chunk + k * GR + lat, GR, 120) for k in range(NSTEP)]
    other += [(chunk + 4 * GR + lat, 136, 120), (chunk + 9 * GR + lat, 136, 60)]
    busy = lambda now: sum(n * min(1.0, max(0.0, (now - t0) / dt)) for t0, dt, n in other)
    tiles = [t for k in range(max(map(len, rest))) for t in TILE_ORDER if k < len(rest[t])]
    end = chunk + NSTEP * GR + 40
    rate = (len(tiles) * work + busy(end)) / end
    free = {x: rate * x[0] - busy(x[0]) for x in slots}
    follow = []
    for i, t in enumerate(tiles):
        x = min((x for x in free if x[1] == t), key=lambda x: abs(free[x] - (i + 0.3) * work))
        del free[x]
        cc, g = rest[t].pop()
        follow.append((cc, t, g) + x[2:])
    return pos, tied, follow


def _dot(a, b):
    return jnp.dot(a, b, preferred_element_type=F32)


def _pad_rows(x, rows):
    return jnp.concatenate([x, jnp.zeros((rows - x.shape[0], x.shape[1]), x.dtype)], axis=0)


def _round_bf16(x):
    return x.astype(BF).astype(F32)


def _norm_bound(sq):
    bits = pltpu.bitcast(sq, I32)
    return pltpu.bitcast(((bits >> 1) + 0x1FC1FFFF) & np.int32(-65536), F32)


def _add_to_first_rows(x, y):
    return jnp.concatenate(
        [x[r:r + 8] + y if r == 0 else x[r:r + 8] for r in range(0, x.shape[0], 8)], axis=0)


def _recip24(x):
    x = jnp.broadcast_to(x, (8, x.shape[1]))
    r = pltpu.reciprocal(x, approx=True)
    return jnp.concatenate([r * (2.0 - x * r)] * 3, axis=0)


def _join_heads(o):
    row = lax.broadcasted_iota(I32, (8, o[0].shape[1]), 0)
    return jnp.concatenate(
        [o[0][0:16], jnp.where(row < 2, o[0][16:24], o[1][0:8]),
         o[1][8:16], jnp.where(row < 4, o[1][16:24], o[2][0:8]),
         o[2][8:16], jnp.where(row < 6, o[2][16:24], o[3][0:8]),
         o[3][8:24]], axis=0)


def _at(start, size):
    if isinstance(start, int):
        return pl.ds(start, size)
    return pl.ds(pl.multiple_of(start, min(size, L)), size)


def _kernel(xa_hbm, wq_hbm, wkt_hbm, wvt_hbm, woa_hbm, xb_hbm, wqkv_hbm, wob_hbm, out_hbm,
            xa, xb, wq, woa, wqkv, wob, wqt, wbg, wot, xbp,
            qa, kat, ka, kbc, va, p_a, oa,
            qb, kb, vb, s_b, p_b, m_b, ob, ob2, qmask,
            obuf, wkt, wvt, in_sem, out_sem):
    pos, tied, follow = _schedule()
    vpu_groups = sorted({cc % NCH * 8 + g for cc in range(NCC)
                         for t in range(NT) for g in pos[cc][t]})
    vpu_slot = {grp: i for i, grp in enumerate(vpu_groups)}

    k1 = 3 * L
    parts = [[(wkt_hbm, wkt), (wvt_hbm, wvt),
              (xa_hbm.at[0:k1, 0:NB], xa.at[0:k1, 0:NB]), (wq_hbm.at[0:k1], wq.at[0:k1])],
             [(xa_hbm.at[k1:D, 0:NB], xa.at[k1:D, 0:NB]), (wq_hbm.at[k1:D], wq.at[k1:D]),
              (xa_hbm.at[:, NB:2 * NB], xa.at[:, NB:2 * NB])],
             [(xa_hbm.at[:, 2 * NB:S], xa.at[:, 2 * NB:S])],
             [(xb_hbm, xb), (wqkv_hbm, wqkv)],
             [(woa_hbm, woa), (wob_hbm, wob)]]
    loads = []
    for part in parts:
        first = sum(map(len, loads))
        loads.append([pltpu.make_async_copy(src, dst, in_sem.at[first + i])
                      for i, (src, dst) in enumerate(part)])

    def request(i):
        for c in loads[i]:
            c.start()

    def arrived(i):
        for c in loads[i]:
            c.wait()

    request(0)
    request(1)
    request(2)
    arrived(0)
    wkv = jnp.concatenate([_pad_rows(wkt[...].astype(F32), 24),
                           _pad_rows(wvt[...].astype(F32), 24)], axis=0).astype(BF)
    row24 = lax.broadcasted_iota(I32, (24, NB), 0)
    row8 = lax.broadcasted_iota(I32, (8, L), 0)

    def first_block_part(lo, hi):
        x = xa[lo:hi, 0:NB]
        out = [_dot(wkv[:, lo:hi], x)]
        for r in range(0, D, L):
            lhs = wq[lo:hi, r:min(r + L, D)].T
            wqt[r:min(r + L, D), lo:hi] = lhs
            out.append(_dot(lhs, x))
        return jnp.concatenate(out, axis=0)

    def store_kv(n, r):
        cols = pl.ds(n * NB, NB)
        kt = _round_bf16(r[0:24] * SCALE)
        kat[:, cols] = kt
        v = r[24:48]
        for j in range(4):
            vj = jnp.concatenate([v[24 - 2 * j:24], v[0:24 - 2 * j]], axis=0) if j else v
            va[pl.ds(32 * j, 24), cols] = jnp.where(row24 == ONES_ROW[j], 1.0, vj)
        return jnp.max(jnp.sum(kt * kt, axis=0, keepdims=True), axis=1, keepdims=True)

    def store_q(n, r):
        for h in range(H):
            q = _pad_rows(r[h * DH:(h + 1) * DH], 24)
            qn = _norm_bound(jnp.broadcast_to(jnp.sum(q * q, axis=0, keepdims=True), (8, NB)))
            qa[n * H + h, 0:24, :] = jnp.concatenate(
                [q[0:16], jnp.where(row24[0:8] == DH - 16, qn, q[16:24])], axis=0)

    def project_kv(n):
        return store_kv(n, _dot(wkv, xa[:, pl.ds(n * NB, NB)]))

    def project_q(n):
        x = xa[:, pl.ds(n * NB, NB)]
        store_q(n, jnp.concatenate(
            [_dot(wqt[r:min(r + L, D), :], x) for r in range(0, D, L)], axis=0))

    s_b[0:48 + D, :] = first_block_part(0, k1)
    arrived(1)
    request(3)
    head = s_b[0:48 + D, :] + first_block_part(k1, D)
    k2 = [store_kv(0, head[0:48])]
    store_q(0, head[48:])
    k2.append(project_kv(1))
    project_q(1)
    arrived(2)
    request(4)
    k2 += [project_kv(n) for n in range(2, NBLK)]
    shift = -_norm_bound(jnp.broadcast_to(functools.reduce(jnp.maximum, k2), (8, L)))
    for n in range(NBLK):
        kt = jnp.where(row24 == DH, jnp.tile(shift, (3, NT)), kat[:, pl.ds(n * NB, NB)])
        kn = _pad_rows(kt, L).T
        ka[pl.ds(n * NB // 2, NB // 2), :] = pltpu.bitcast(kn[:, 0:32].astype(BF), I32)
    for n in range(NBLK):
        kn = _pad_rows(_round_bf16(kat[:, pl.ds(n * NB, NB)]), L).T
        for grp in range(n * NB // 16, (n + 1) * NB // 16):
            if grp in vpu_slot:
                rows = kn[grp * 16 - n * NB:grp * 16 - n * NB + 16]
                for d in range(DH):
                    kbc[vpu_slot[grp], d] = jnp.broadcast_to(rows[:, d:d + 1], (16, L))
    kat[:, 0:NB] = jnp.zeros((24, NB), F32)
    zero = lambda width=L: kat[0:8, 0:width]
    for n in range(2, NBLK):
        project_q(n)

    def q_tile(u, t):
        return _pad_rows(qa[u, 0:24, pl.ds(t * L, L)], 32)

    def q_row(u, d, t):
        return jnp.broadcast_to(qa[u, pl.ds(d, 1), pl.ds(t * L, L)], (8, L))

    def p_tile(cc, g, t):
        return pl.ds(cc * 64 + g * 8, 8), pl.ds(t * L, L)

    def vpu_probs(u, grp, tiles, after=None):
        acc = {t: [q_row(u, DH, t) * shift] * 2 for t in tiles}
        if after is not None:
            acc = {t: [jnp.where(zero() != 0.0, after, a[0]), a[0]] for t, a in acc.items()}
        for d in range(DH):
            kk = kbc[vpu_slot[grp], d]
            for t in tiles:
                qq = q_row(u, d, t)
                acc[t] = [acc[t][0] + kk[0:8] * qq, acc[t][1] + kk[8:16] * qq]
        return {t: jnp.exp2(jnp.concatenate(acc[t], axis=0)) for t in tiles}

    def make_probs(u, q, cc, on_vpu, later, after=()):
        c = cc % NCH
        scores = []
        for t in range(NT):
            rows = [ka[pl.ds(c * 64 + g * 8, 8), :] for g in range(8) if g not in on_vpu[t]]
            mine = [x for tt, x in after if tt == t]
            for i, x in enumerate(mine):
                i = (2 * i + 1) * len(rows) // (2 * len(mine))
                rows[i] = rows[i] | (pltpu.bitcast(zero(), I32) & x)[:, 0:32]
            scores.append(_dot(pltpu.bitcast(jnp.concatenate(rows, axis=0), BF), q[t]))
        side = {g: vpu_probs(u, c * 8 + g,
                             [t for t in range(NT) if g in on_vpu[t] and (t, g) not in later])
                for g in range(8) if any(g in x for x in on_vpu)}
        for t in range(NT):
            n = 0
            for g in range(8):
                if (t, g) in later:
                    continue
                if g in on_vpu[t]:
                    p = side[g][t]
                else:
                    p = jnp.exp2(scores[t][n * 16:(n + 1) * 16])
                    n += 1
                p_a[p_tile(cc, g, t)] = pltpu.bitcast(p.astype(BF), I32)
        return scores

    def make_later_probs(u, tiles, scores, steps):
        for cc, t, g, kind, k, r in tiles:
            x = scores[k][t] if kind == "k" else steps[k][:, t * L:(t + 1) * L]
            r = min(8 * r, x.shape[0] - 8)
            p = vpu_probs(u + cc // NCH, cc % NCH * 8 + g, [t], x[r:r + 8])[t]
            p_a[p_tile(cc, g, t)] = pltpu.bitcast(p.astype(BF), I32)

    def use_probs(cc, acc, loaded):
        j, c = divmod(cc, NCH)
        for t in range(NT):
            p = jnp.concatenate([loaded[t, g] if (t, g) in loaded else p_a[p_tile(cc, g, t)]
                                 for g in range(8)], axis=0)
            o = _dot(va[pl.ds(32 * j, 24), pl.ds(c * L, L)], pltpu.bitcast(p, BF))
            acc[t] = _add_to_first_rows(o, zero()) if c == 0 else acc[t] + o

    def finish(u, j, acc, bad):
        oa[u] = jnp.concatenate(acc, axis=1)
        r = ONES_ROW[j]
        for t in range(NT):
            a = acc[t][r // 8 * 8:r // 8 * 8 + 8]
            ok = (a >= MIN_DENOM) & (a <= MAX_DENOM)
            bad = jnp.where(ok | (row8 != r % 8), bad, 1.0)
        return bad

    def project_b_steps(i):
        g, n = i >> 2, i & 3
        cols = pl.ds(pl.multiple_of(n * NB, NB), NB)
        acc = {}

        def step(part, kt):
            lo, hi = kt * L, min(kt * L + L, D)
            x = pltpu.bitcast(xbp[lo // 2:hi // 2, cols], BF)
            o = _dot(wbg[g, part * GR:(part + 1) * GR, lo:hi], x)
            r = acc[part] = _add_to_first_rows(o, zero(NB)) if kt == 0 else acc[part] + o
            if hi == D and part == 0:
                rows = pl.ds(pl.multiple_of(g * KROWS + 48 + n * (NB // 2), 16), NB // 2)
                kb[rows, 0:L] = pltpu.bitcast(_pad_rows(r, L).T.astype(BF), I32)
            elif hi == D and part == 1:
                qb[pl.ds(pl.multiple_of(g * 40, 8), 40), cols] = pltpu.bitcast(
                    _pad_rows(r * SCALE, 80).astype(BF), I32)
            elif hi == D:
                vb[g, :, cols] = r
            return o

        return [functools.partial(step, part, kt) for part in range(3) for kt in range(5)]

    def first_units():
        wt = {}

        def transpose(r):
            wt[r] = wqkv[:, r * L:min(r * L + L, 3 * D)].T.astype(F32)
            full = jnp.concatenate([wt[i] for i in sorted(wt)], axis=0)
            for part, r0 in enumerate((D, 0, 2 * D)):
                for g in range(G):
                    lo = r0 + g * GR
                    if (lo + GR - 1) // L == r:
                        wbg[g, part * GR:(part + 1) * GR, 0:D] = full[lo:lo + GR]
            return pltpu.bitcast(wt[r][-8:, 3 * L:4 * L], I32)

        def repack(r):
            x = pltpu.bitcast(xb[r * 16:r * 16 + 16, :], I32)
            xbp[r * 8:r * 8 + 8, :] = x
            return functools.reduce(jnp.bitwise_and, [x[:, i:i + L] for i in range(0, S, L)])

        jobs = []
        nw, nx = pl.cdiv(3 * D, L), D // 16
        for r in range(nw):
            jobs.append(functools.partial(transpose, r))
            jobs += [functools.partial(repack, i)
                     for i in range(r * nx // nw, (r + 1) * nx // nw)]
        for g in range(G):
            kb[g * KROWS:g * KROWS + 48, 0:L] = jnp.zeros((48, L), I32)
        on_vpu = [[[] for _ in range(NT)] for _ in range(NCC)]
        later = []
        for cc in range(NCC):
            n = (cc + 1) * VPU_FIRST // NCC - cc * VPU_FIRST // NCC
            for k in range(n):
                t = len(later) % NT
                g = min(g for g in range(8)
                        if cc % NCH * 8 + g in vpu_slot and g not in on_vpu[cc][t])
                on_vpu[cc][t].append(g)
                later.append((cc, t, g, "k", cc, (2 * k + 1) * 7 // n))
        arrived(3)
        scores = []
        after = []
        for j in range(U):
            q = [q_tile(j, t).astype(BF) for t in range(NT)]
            for cc in range(j * NCH, (j + 1) * NCH):
                scores.append(make_probs(
                    j, q, cc, on_vpu[cc], [x[1:3] for x in later if x[0] == cc], after))
                todo = jobs[cc * len(jobs) // (NCC - 1):(cc + 1) * len(jobs) // (NCC - 1)]
                after = [((cc + i) % NT, job()) for i, job in enumerate(todo)]
        make_later_probs(0, later, scores, None)

    def middle_units(i, bad):
        steps = project_b_steps(i)
        loaded = {}
        scores = []
        for j in range(U):
            u = i * U + j
            q = [q_tile(u + U, t).astype(BF) for t in range(NT)]
            acc = [None] * NT
            for cc in range(j * NCH, (j + 1) * NCH):
                use_probs(cc, acc, loaded)
                loaded = {(t, g): p_a[p_tile(cc + 1, g, t)] for _, t, g in tied.get(cc, [])}
                qc = list(q)
                for k, t, g in tied.get(cc, []):
                    w = q_tile(u + U, t)
                    none = loaded[t, g] & pltpu.bitcast(zero(), I32)
                    qc[t] = jnp.concatenate(
                        [pltpu.bitcast(pltpu.bitcast(w[r:r + 8], I32) | none, F32)
                         if r == k * 16 else w[r:r + 8] for r in range(0, 32, 8)],
                        axis=0).astype(BF)
                scores.append(make_probs(
                    u + U, qc, cc, pos[cc], [x[1:3] for x in follow if x[0] == cc]))
            if j == U - 1:
                steps = [step() for step in steps]
            bad = finish(u, j, acc, bad)
        make_later_probs((i + 1) * U, follow, scores, steps)
        return bad

    first_units()
    bad = lax.fori_loop(0, UNITS // U - 1, middle_units, jnp.zeros((8, L), F32))

    def lane(rows):
        return lax.broadcasted_iota(I32, (rows, L), 1)

    def row(rows):
        return lax.broadcasted_iota(I32, (rows, L), 0)

    for u in range(4):
        lo = (((lane(40) >> 5) + u) & 3) * (DH // 2)
        qmask[u] = jnp.where((row(40) >= lo) & (row(40) < lo + DH // 2), -1, 0)

    def first_block(t):
        return max(0, 5 - 4 * t) if isinstance(t, int) else 0

    def scores_b(g, t):
        l16 = lane(16)
        slot = ((l16 >= DH).astype(I32) + (l16 >= 2 * DH).astype(I32)
                + (l16 >= 3 * DH).astype(I32))
        odd = (slot & 1) == 1
        q = qb[pl.ds(pl.multiple_of(g * 40, 8), 40), pl.ds(t * L, L)]
        qs = [pltpu.bitcast(_pad_rows(q & qmask[u], L // 2), BF) for u in range(4)]
        keys = {}
        half = {}

        def key(i):
            if i not in keys:
                start = pl.multiple_of(g * KROWS + (4 * t - 5 + i) * 16, 16)
                keys[i] = kb[pl.ds(start, 16), 0:L]
            return keys[i]

        def shifted(parity, i):
            if (parity, i) not in half:
                a, b = (key(i + 1), key(i)) if parity == 0 else (key(i), key(i + 1))
                half[parity, i] = jnp.where(odd, a, b)
            return half[parity, i]

        mx = [None] * 4

        def part(c):
            if c:
                return
            blocks = range(8, first_block(t) - 1, -1)
            for u in range(4):
                two = ((slot - u) & 2) == 2
                k = jnp.concatenate([jnp.where(two, shifted(u & 1, i + 2), shifted(u & 1, i))
                                     for i in blocks], axis=0)
                s = _dot(pltpu.bitcast(k, BF), qs[u])
                for n, i in enumerate(blocks):
                    si = s[32 * n:32 * n + 32]
                    if i == 0:
                        si = jnp.where((lane(32) & 31) < row(32), si, NEG)
                    elif i == 8:
                        si = jnp.where((lane(32) & 31) >= row(32), si, NEG)
                    elif i < 8 - 4 * t:
                        si = jnp.where((lane(32) >> 5) >= 8 - 4 * t - i, si, NEG)
                    s_b[pl.ds(t * 288 + 32 * i, 32), pl.ds(u * L, L)] = si
                    mc = jnp.max(si.reshape(4, 8, L), axis=0)
                    mx[u] = mc if mx[u] is None else jnp.maximum(mx[u], mc)

        def done():
            for u in range(4):
                m_b[pl.ds(t * 8, 8), pl.ds(u * L, L)] = jnp.broadcast_to(
                    jnp.max(mx[u], axis=0, keepdims=True), (8, L))

        return part, done

    def probs_b(t, slot=None):
        m = [m_b[_at(t * 8, 8), pl.ds(u * L, L)] for u in range(4)]
        dst, base = (p_b, t) if slot is None else (p_a, slot)

        def part(c):
            for i in ((0,), (4, 3, 2, 1), (8, 7, 6, 5))[c]:
                if i >= first_block(t):
                    for u in range(4):
                        s = s_b[_at(t * 288 + 32 * i, 32), pl.ds(u * L, L)]
                        p = jnp.exp2(s - jnp.concatenate([m[u]] * 4, axis=0)).astype(BF)
                        dst[_at(base * 144 + 16 * i, 16), pl.ds(u * L, L)] = (
                            pltpu.bitcast(p, I32))

        return part, lambda: None

    def values_b(g, t, out=None, slot=None):
        b0 = ((lane(16) >> 5) & 1) == 1
        b1 = ((lane(16) >> 5) & 2) == 2
        nothing = jnp.zeros((16, L), I32)
        src, base = (p_b, t) if slot is None else (p_a, slot)
        probs = {}
        half = {}

        def prob(u, i):
            if not first_block(t) <= i < 9:
                return nothing
            if (u, i) not in probs:
                probs[u, i] = src[_at(base * 144 + 16 * i, 16), pl.ds(u * L, L)]
            return probs[u, i]

        def shifted(u, i):
            if not first_block(t) <= i < 10:
                return nothing
            if (u, i) not in half:
                half[u, i] = jnp.where(b0, prob((u - 1) % 4, i - 1), prob(u, i))
            return half[u, i]

        acc = [None] * 4

        def part(c):
            if isinstance(t, int) and t - 2 + c < 0:
                return
            for j in range(4):
                p = jnp.concatenate(
                    [jnp.where(b1, shifted((j - 2) % 4, i - 2), shifted(j, i))
                     for i in range(4 * c, 4 * c + 4)], axis=0)
                v = [vb[g, pl.ds(16 * j + 8 * i, 8), _at((t - 2 + c) * L, L)] for i in range(3)]
                r = ONES_ROW[j]
                v[r // 8] = jnp.where(row8 == r % 8, 1.0, v[r // 8])
                o = _dot(jnp.concatenate(v, axis=0), pltpu.bitcast(p, BF))
                acc[j] = o + (kat[:, pl.ds(j * L, L)] if acc[j] is None else acc[j])

        def done():
            o = _join_heads([a * _recip24(a[r:r + 1]) for a, r in zip(acc, ONES_ROW)])
            if out is None:
                ob[g, :, _at(t * L, L)] = o
            else:
                ob2[out[0], :, pl.ds(out[1] * L, L)] = o

        return part, done

    def run(*stages):
        for c in (2, 1, 0):
            for part, _ in stages:
                part(c)
        for _, done in stages:
            done()

    steps = project_b_steps(UNITS // U - 1)
    for j in range(U):
        acc = [None] * NT
        for cc in range(j * NCH, (j + 1) * NCH):
            use_probs(cc, acc, {})
            if cc % 4 == 3 and cc // 4 < NSTEP:
                steps[cc // 4]()
            if cc % 4 == 1:
                run(scores_b(0, cc // 4))
        bad = finish(UNITS - U + j, j, acc, bad)

    @pl.when(jnp.max(bad) > 0.0)
    def _():
        def exact(u, carry):
            kbc[u, 0] = jnp.zeros((16, L), F32)
            q = _pad_rows(jnp.where(row24 == DH, 0.0, qa[u, 0:24]), 32).astype(BF)

            def scores(c, mx):
                k = pltpu.bitcast(ka[pl.ds(pl.multiple_of(c * 256, 256), 256), :], BF)
                s = _dot(k, q)
                p_a[pl.ds(pl.multiple_of(c * 512, 512), 512), :] = pltpu.bitcast(s, I32)
                return jnp.maximum(mx, jnp.max(s, axis=0, keepdims=True))

            m = lax.fori_loop(0, S // 512, scores, jnp.full((1, NB), -jnp.inf, F32))

            def values(c, acc):
                keys = pl.ds(pl.multiple_of(c * 512, 512), 512)
                p = jnp.exp2(pltpu.bitcast(p_a[keys, :], F32) - m).astype(BF)
                return acc + _dot(va[pl.ds(pl.multiple_of((u & 3) * 32, 32), 24), keys], p)

            oa[u] = lax.fori_loop(0, S // 512, values, jnp.zeros((24, NB), F32))
            return carry

        lax.fori_loop(0, UNITS, exact, 0)

    for t in range(NCH):
        run(probs_b(t), scores_b(1, t))

    def middle_groups(g, carry):
        for t in range(NCH):
            run(values_b(g, t), probs_b(t), scores_b(g + 2, t))
        return carry

    lax.fori_loop(0, G - 2, middle_groups, 0)

    arrived(4)

    def last_groups(n, buf):
        jobs = []
        for i in range(2):
            t, slot = 2 * n + i, 2 * buf + i
            jobs.append(lambda t=t, slot=slot: run(values_b(G - 2, t, (0, slot)),
                                                   probs_b(t, slot)))
            jobs.append(lambda t=t, slot=slot: run(values_b(G - 1, t, (1, slot), slot)))
        return jobs

    def out_block(n, buf, first=False, last=False):
        cols = _at(n * OUT_NB, OUT_NB)
        u0 = (n >> 1) * H
        sub = _at((n & 1) * OUT_NB, OUT_NB)
        heads_b = lambda: jnp.concatenate(
            [ob[g, :, cols] for g in range(G - 2)]
            + [ob2[g, :, pl.ds(buf * OUT_NB, OUT_NB)] for g in range(2)], axis=0).astype(BF)
        b = None if first else heads_b()
        a = jnp.concatenate(
            [_join_heads([oa[u0 + 4 * g + j, :, sub]
                          * _recip24(oa[u0 + 4 * g + j, pl.ds(ONES_ROW[j], 1), sub])
                          for j in range(4)]) for g in range(G)], axis=0).astype(BF)
        wt = wot
        if first:
            wt = jnp.concatenate([w[:, r:min(r + L, D)].T
                                  for w in (woa, wob) for r in range(0, D, L)], axis=0)
            wot[...] = wt
        side = (last_groups(n, buf) if first else []) + (
            [] if last else last_groups(n + 1, 1 - buf))
        tiles = range(2 * D // L)
        for i, j in enumerate(tiles if first else reversed(tiles)):
            for job in side[i:i + 1] if first else side[i // 2:i // 2 + i % 2]:
                job()
            r0, r1 = j * L, (j + 1) * L
            lhs = wt[r0:r1, :]
            res = []
            if r0 < D:
                res.append(_dot(lhs[0:min(r1, D) - r0], a))
            if r1 > D:
                b = heads_b() if b is None else b
                res.append(_dot(lhs[max(r0, D) - r0:L], b))
            obuf[cols, r0:r1] = jnp.concatenate(res, axis=0).T.astype(BF)

    def out_copy(i, n, count):
        rows = _at(n * OUT_NB, count * OUT_NB)
        return pltpu.make_async_copy(obuf.at[rows], out_hbm.at[rows], out_sem.at[i])

    nout = S // OUT_NB
    nmid = nout // 2 - 1
    out_block(0, 1, first=True)
    out_copy(nmid, 0, 1).start()

    def middle_blocks(i, carry):
        out_block(1 + 2 * i, 0)
        out_block(2 + 2 * i, 1)
        out_copy(i, 1 + 2 * i, 2).start()
        return carry

    lax.fori_loop(0, nmid, middle_blocks, 0)
    out_block(nout - 1, 0, last=True)
    out_copy(nmid + 1, nout - 1, 1).start()
    out_copy(nmid, 0, 1).wait()
    for i in range(nmid):
        out_copy(i, 1 + 2 * i, 2).wait()
    out_copy(nmid + 1, nout - 1, 1).wait()


@jax.jit
def pallas_concat_heads__grouped_kv_mqa__sliding_block__prompt_kernel(
    A_x: jax.Array,
    A_wq: jax.Array,
    A_wk: jax.Array,
    A_wv: jax.Array,
    A_wo: jax.Array,
    B_x: jax.Array,
    B_wqkv: jax.Array,
    B_wo: jax.Array,
):
    hbm = pl.BlockSpec(memory_space=pltpu.HBM)
    vmem = pltpu.VMEM
    scratch = [
        vmem((D, S), BF), vmem((D, S), BF),
        vmem((D, D), BF), vmem((D, D), BF),
        vmem((D, 3 * D), BF), vmem((D, D), BF),
        vmem((D, D), BF), vmem((G, 256, 5 * L), F32),
        vmem((2 * D, D), BF), vmem((D // 2, S), I32),
        vmem((UNITS, 32, NB), F32), vmem((24, S), F32),
        vmem((S // 2, 32), I32), vmem((UNITS, DH, 16, L), F32),
        vmem((128, S), F32), vmem((U * S // 2, NB), I32),
        vmem((UNITS, 24, NB), F32),
        vmem((G * 40, S), I32), vmem((G * KROWS, 2 * L), I32),
        vmem((G, GR, S), F32), vmem((NCH * 288, NB), F32),
        vmem((NCH * 144, NB), I32), vmem((NCH * 8, NB), F32),
        vmem((G - 2, GR, S), F32), vmem((2, GR, 2 * OUT_NB), F32),
        vmem((4, 40, L), I32), vmem((S, 2 * D), BF),
        vmem((DH, D), BF), vmem((DH, D), BF),
        pltpu.SemaphoreType.DMA((12,)), pltpu.SemaphoreType.DMA((S // OUT_NB // 2 + 1,)),
    ]
    out = pl.pallas_call(
        _kernel,
        in_specs=[hbm] * 8,
        out_specs=hbm,
        out_shape=jax.ShapeDtypeStruct((S, 2 * D), BF),
        scratch_shapes=scratch,
        compiler_params=pltpu.CompilerParams(vmem_limit_bytes=110 * 2**20),
        name="fused_attention",
    )(A_x.reshape(S, D).T, A_wq, A_wk.T, A_wv.T, A_wo, B_x.reshape(S, D).T, B_wqkv, B_wo)
    return out.reshape(1, S, 2 * D)
```

```python
import functools
import math

import jax
import jax.numpy as jnp
import numpy as np
from jax import lax
import jax.experimental.pallas as pl
import jax.experimental.pallas.tpu as pltpu

S = 2048
D = 576
H = 32
DH = D // H
L = 128
NT = 4
NB = NT * L
NBLK = S // NB
NCH = S // L
UNITS = NBLK * H
U = 4
NCC = U * NCH
G = H // 4
GR = 4 * DH
KROWS = S // 2 + 48
NSTEP = 15
OUT_NB = 256
ONES_ROW = (18, 0, 0, 0)
SCALE = float(DH ** -0.5 * math.log2(math.e))
NEG = -1e30
MIN_DENOM = 2.0 ** -80
MAX_DENOM = 2.0 ** 12

BF = jnp.bfloat16
F32 = jnp.float32
I32 = jnp.int32

TILE_ORDER = (2, 3, 0, 1)
VPU_SLOTS = (
    0, 1, 3, 3, 6, 10, 10, 14, 16, 17, 18, 20, 23, 25, 27, 28, 30, 32, 34, 35, 37, 39, 41,
    43, 45, 47, 48, 50, 53, 55, 57, 58, 61, 63, 65, 67, 68, 70, 72, 74, 76, 77, 79, 82, 84,
    85, 86, 87, 90, 93, 96, 96, 98, 100, 102, 104, 106, 108, 109, 112, 114, 115, 117, 119,
    122, 123, 125, 126, 128, 130, 133, 135, 137, 139, 141, 143, 145, 147, 148, 150, 153,
    155, 156, 157)
VPU_FIRST = 190


def _schedule():
    picks = [(TILE_ORDER[i % NT], x // 10, x % 10) for i, x in enumerate(VPU_SLOTS)]
    used = {(c, 7 - k) for _, c, k in picks if k < 8}
    pos = [[[] for _ in range(NT)] for _ in range(NCC)]
    tied = {}
    rest = [[] for _ in range(NT)]

    def free_group(cc, tiles):
        groups = [g for g in range(8) if all(g not in pos[cc][t] for t in tiles)]
        g = min(groups, key=lambda g: ((cc % NCH, g) not in used, g))
        used.add((cc % NCH, g))
        for t in tiles:
            pos[cc][t].append(g)
        return g

    for t, c, k in sorted(picks, key=lambda x: x[2] >= 8):
        for cc in range(c, NCC, NCH):
            if k < 8:
                pos[cc][t].append(7 - k)
                if cc == 0:
                    rest[t].append((cc, 7 - k))
            elif 0 < cc < NCC - 1:
                tied.setdefault(cc, []).append((9 - k, t, free_group(cc + 1, [t])))
            else:
                rest[t].append(((cc + 1) % NCC, free_group((cc + 1) % NCC, [t])))
    for cc in range(NCC):
        if cc % 8 == 4 or cc == 0:
            g = free_group(cc, range(NT))
            for t in range(NT):
                rest[t].append((cc, g))

    chunk, lat, work = 129, 95, 75
    skew = lambda t: 4 * ((0.0, 0.1, 0.5, 0.6)[(t + 2) % NT] + 0.6)
    slots = [(24 + lat - chunk + 8 * r + skew(t), t, "k", NCC - 2, r)
             for r in range(2, 12) for t in range(NT)]
    slots += [(24 + lat + 8 * r + skew(t), t, "k", NCC - 1, r)
              for r in range(12) for t in range(NT)]
    slots += [(chunk + k * GR + lat + 8 * r + skew(t), t, "s", k, r)
              for k in range(NSTEP) for r in range(GR // 8) for t in range(NT)]
    other = [(0, chunk, 108), (chunk, lat, 108 * lat / chunk)]
    other += [(chunk + k * GR + lat, GR, 105) for k in range(NSTEP)]
    other += [(chunk + 4 * GR + lat, 136, 120), (chunk + 9 * GR + lat, 136, 60)]
    busy = lambda now: sum(n * min(1.0, max(0.0, (now - t0) / dt)) for t0, dt, n in other)
    tiles = [t for k in range(max(map(len, rest))) for t in TILE_ORDER if k < len(rest[t])]
    end = chunk + NSTEP * GR + 60
    rate = (len(tiles) * work + busy(end)) / end
    free = {x: rate * x[0] - busy(x[0]) for x in slots}
    follow = []
    for i, t in enumerate(tiles):
        x = min((x for x in free if x[1] == t), key=lambda x: abs(free[x] - i * work))
        del free[x]
        cc, g = rest[t].pop()
        follow.append((cc, t, g) + x[2:])
    return pos, tied, follow


def _runs(single):
    cuts = sorted({0, 8, *single, *(g + 1 for g in single)})
    return [(a, b - a) for a, b in zip(cuts, cuts[1:])]


def _dot(a, b):
    return jnp.dot(a, b, preferred_element_type=F32)


def _pad_rows(x, rows):
    return jnp.concatenate([x, jnp.zeros((rows - x.shape[0], x.shape[1]), x.dtype)], axis=0)


def _round_bf16(x):
    return x.astype(BF).astype(F32)


def _norm_bound(sq):
    bits = pltpu.bitcast(sq, I32)
    return pltpu.bitcast(((bits >> 1) + 0x1FC1FFFF) & np.int32(-65536), F32)


def _add_to_first_rows(x, y):
    return jnp.concatenate(
        [x[r:r + 8] + y if r == 0 else x[r:r + 8] for r in range(0, x.shape[0], 8)], axis=0)


def _recip24(x):
    x = jnp.broadcast_to(x, (8, x.shape[1]))
    r = pltpu.reciprocal(x, approx=True)
    return jnp.concatenate([r * (2.0 - x * r)] * 3, axis=0)


def _join_heads(o):
    row = lax.broadcasted_iota(I32, (8, o[0].shape[1]), 0)
    return jnp.concatenate(
        [o[0][0:16], jnp.where(row < 2, o[0][16:24], o[1][0:8]),
         o[1][8:16], jnp.where(row < 4, o[1][16:24], o[2][0:8]),
         o[2][8:16], jnp.where(row < 6, o[2][16:24], o[3][0:8]),
         o[3][8:24]], axis=0)


def _at(start, size):
    if isinstance(start, int):
        return pl.ds(start, size)
    return pl.ds(pl.multiple_of(start, min(size, L)), size)


def _kernel(xa_hbm, wq_hbm, wkt_hbm, wvt_hbm, woa_hbm, xb_hbm, wqkv_hbm, wob_hbm, out_hbm,
            xa, xb, wq, woa, wqkv, wob, wqt, wbg, wot, xbp,
            qa, kat, ka, kbc, va, p_a, oa,
            qb, kb, vb, s_b, p_b, m_b, ob, ob2, qmask,
            obuf, wkt, wvt, in_sem, out_sem):
    pos, tied, follow = _schedule()
    vpu_groups = sorted({cc % NCH * 8 + g for cc in range(NCC)
                         for t in range(NT) for g in pos[cc][t]})
    vpu_slot = {grp: i for i, grp in enumerate(vpu_groups)}

    k1 = 3 * L
    parts = [[(wkt_hbm, wkt), (wvt_hbm, wvt),
              (xa_hbm.at[0:k1, 0:NB], xa.at[0:k1, 0:NB]), (wq_hbm.at[0:k1], wq.at[0:k1])],
             [(xa_hbm.at[k1:D, 0:NB], xa.at[k1:D, 0:NB]), (wq_hbm.at[k1:D], wq.at[k1:D]),
              (xa_hbm.at[:, NB:2 * NB], xa.at[:, NB:2 * NB])],
             [(xa_hbm.at[:, 2 * NB:S], xa.at[:, 2 * NB:S])],
             [(xb_hbm, xb), (wqkv_hbm, wqkv)],
             [(woa_hbm, woa), (wob_hbm, wob)]]
    loads = []
    for part in parts:
        first = sum(map(len, loads))
        loads.append([pltpu.make_async_copy(src, dst, in_sem.at[first + i])
                      for i, (src, dst) in enumerate(part)])

    def request(i):
        for c in loads[i]:
            c.start()

    def arrived(i):
        for c in loads[i]:
            c.wait()

    request(0)
    request(1)
    request(2)
    arrived(0)
    wkv = _pad_rows(jnp.concatenate([wkt[...].astype(F32), wvt[...].astype(F32)], axis=0), 40)
    row24 = lax.broadcasted_iota(I32, (24, NB), 0)
    row8 = lax.broadcasted_iota(I32, (8, L), 0)

    def first_block_part(lo, hi):
        x = xa[lo:hi, 0:NB]
        out = [_dot(wkv[:, lo:hi], x)]
        for r in range(0, D, L):
            lhs = wq[lo:hi, r:min(r + L, D)].T
            wqt[r:min(r + L, D), lo:hi] = lhs
            out.append(_dot(lhs, x))
        return jnp.concatenate(out, axis=0)

    def store_kv(n, r):
        cols = pl.ds(n * NB, NB)
        kt = _round_bf16(_pad_rows(r[0:DH], 24) * SCALE)
        kat[:, cols] = kt
        v = _pad_rows(r[DH:2 * DH], 24)
        for j in range(4):
            vj = jnp.concatenate([v[24 - 2 * j:24], v[0:24 - 2 * j]], axis=0) if j else v
            va[pl.ds(32 * j, 24), cols] = jnp.where(row24 == ONES_ROW[j], 1.0, vj)
        return jnp.max(jnp.sum(kt * kt, axis=0, keepdims=True), axis=1, keepdims=True)

    def store_q(n, r):
        for h in range(H):
            q = _pad_rows(r[h * DH:(h + 1) * DH], 24)
            qn = _norm_bound(jnp.broadcast_to(jnp.sum(q * q, axis=0, keepdims=True), (8, NB)))
            qa[n * H + h, 0:24, :] = jnp.concatenate(
                [q[0:16], jnp.where(row24[0:8] == DH - 16, qn, q[16:24])], axis=0)

    def project_kv(n):
        return store_kv(n, _dot(wkv, xa[:, pl.ds(n * NB, NB)]))

    def project_q(n):
        x = xa[:, pl.ds(n * NB, NB)]
        store_q(n, jnp.concatenate(
            [_dot(wqt[r:min(r + L, D), :], x) for r in range(0, D, L)], axis=0))

    s_b[0:40 + D, :] = first_block_part(0, k1)
    arrived(1)
    request(3)
    head = s_b[0:40 + D, :] + first_block_part(k1, D)
    k2 = [store_kv(0, head[0:40])]
    store_q(0, head[40:])
    k2.append(project_kv(1))
    project_q(1)
    arrived(2)
    request(4)
    k2 += [project_kv(n) for n in range(2, NBLK)]
    shift = -_norm_bound(jnp.broadcast_to(functools.reduce(jnp.maximum, k2), (8, L)))
    shift24 = jnp.concatenate([jnp.concatenate([shift] * NT, axis=1)] * 3, axis=0)
    for n in range(NBLK):
        kt = jnp.where(row24 == DH, shift24, kat[:, pl.ds(n * NB, NB)])
        kn = _pad_rows(kt, L).T
        ka[pl.ds(n * NB // 2, NB // 2), :] = pltpu.bitcast(kn[:, 0:32].astype(BF), I32)
    for n in range(NBLK):
        kn = _pad_rows(_round_bf16(kat[:, pl.ds(n * NB, NB)]), L).T
        for grp in range(n * NB // 16, (n + 1) * NB // 16):
            if grp in vpu_slot:
                rows = kn[grp * 16 - n * NB:grp * 16 - n * NB + 16]
                for d in range(DH):
                    kbc[vpu_slot[grp], d] = jnp.broadcast_to(rows[:, d:d + 1], (16, L))
    kat[:, 0:NB] = jnp.zeros((24, NB), F32)
    zero = lambda width=L: kat[0:8, 0:width]
    for n in range(2, NBLK):
        project_q(n)

    def q_tile(u, t):
        return _pad_rows(qa[u, 0:24, pl.ds(t * L, L)], 32)

    def p_tile(cc, g, t, count=1):
        return pl.ds(cc * 64 + g * 8, 8 * count), pl.ds(t * L, L)

    def vpu_probs(u, grp, t, after=None):
        q_row = lambda d: qa[u, pl.ds(d, 1), pl.ds(t * L, L)]
        acc = q_row(DH) * shift
        first = acc if after is None else jnp.where(zero() != 0.0, after, acc)
        acc = jnp.concatenate([first, acc], axis=0)
        for d in range(DH):
            acc = acc + kbc[vpu_slot[grp], d] * q_row(d)
        return jnp.exp2(acc)

    def make_probs(u, q, cc, on_vpu, later, after=()):
        c = cc % NCH
        scores = []
        for t in range(NT):
            rows = [ka[pl.ds(c * 64 + g * 8, 8), :] for g in range(8) if g not in on_vpu[t]]
            mine = [x for tt, x in after if tt == t]
            for i, x in enumerate(mine):
                i = (2 * i + 1) * len(rows) // (2 * len(mine))
                rows[i] = rows[i] | (pltpu.bitcast(zero(), I32) & x)[:, 0:32]
            scores.append(_dot(pltpu.bitcast(jnp.concatenate(rows, axis=0), BF), q[t]))
        side = {(t, g): vpu_probs(u, c * 8 + g, t) for g in range(8) for t in range(NT)
                if g in on_vpu[t] and (t, g) not in later}
        for t in range(NT):
            n = 0
            for g, count in _runs(on_vpu[t]):
                if g not in on_vpu[t]:
                    p = jnp.exp2(scores[t][n * 16:(n + count) * 16])
                    n += count
                elif (t, g) in later:
                    continue
                else:
                    p = side[t, g]
                p_a[p_tile(cc, g, t, count)] = pltpu.bitcast(p.astype(BF), I32)
        return scores

    def make_later_probs(u, tiles, scores, steps):
        for cc, t, g, kind, k, r in tiles:
            x = scores[k][t] if kind == "k" else steps[k][:, t * L:(t + 1) * L]
            r = min(8 * r, x.shape[0] - 8)
            p = vpu_probs(u + cc // NCH, cc % NCH * 8 + g, t, x[r:r + 8])
            p_a[p_tile(cc, g, t)] = pltpu.bitcast(p.astype(BF), I32)

    def use_probs(cc, acc, loaded):
        j, c = divmod(cc, NCH)
        for t in range(NT):
            p = jnp.concatenate(
                [loaded[t, g] if (t, g) in loaded else p_a[p_tile(cc, g, t, count)]
                 for g, count in _runs([g for tt, g in loaded if tt == t])], axis=0)
            o = _dot(va[pl.ds(32 * j, 24), pl.ds(c * L, L)], pltpu.bitcast(p, BF))
            acc[t] = _add_to_first_rows(o, zero()) if c == 0 else acc[t] + o

    def finish(u, j, acc, bad):
        oa[u] = jnp.concatenate(acc, axis=1)
        r = ONES_ROW[j]
        for t in range(NT):
            a = acc[t][r // 8 * 8:r // 8 * 8 + 8]
            ok = (a >= MIN_DENOM) & (a <= MAX_DENOM)
            bad = jnp.where(ok | (row8 != r % 8), bad, 1.0)
        return bad

    def project_b_steps(i):
        g, n = i >> 2, i & 3
        cols = pl.ds(pl.multiple_of(n * NB, NB), NB)
        acc = {}

        def step(part, kt):
            lo, hi = kt * L, min(kt * L + L, D)
            x = pltpu.bitcast(xbp[lo // 2:hi // 2, cols], BF)
            o = _dot(wbg[g, part * GR:(part + 1) * GR, lo:hi], x)
            r = acc[part] = _add_to_first_rows(o, zero(NB)) if kt == 0 else acc[part] + o
            if hi == D and part == 0:
                rows = pl.ds(pl.multiple_of(g * KROWS + 48 + n * (NB // 2), 16), NB // 2)
                kb[rows, 0:L] = pltpu.bitcast(_pad_rows(r, L).T.astype(BF), I32)
            elif hi == D and part == 1:
                qb[pl.ds(pl.multiple_of(g * 40, 8), 40), cols] = pltpu.bitcast(
                    _pad_rows(r * SCALE, 80).astype(BF), I32)
            elif hi == D:
                vb[g, :, cols] = r
            return o

        return [functools.partial(step, part, kt) for part in range(3) for kt in range(5)]

    def first_units():
        wt = {}

        def transpose(r):
            wt[r] = wqkv[:, r * L:min(r * L + L, 3 * D)].T.astype(F32)
            full = jnp.concatenate([wt[i] for i in sorted(wt)], axis=0)
            for part, r0 in enumerate((D, 0, 2 * D)):
                for g in range(G):
                    lo = r0 + g * GR
                    if (lo + GR - 1) // L == r:
                        wbg[g, part * GR:(part + 1) * GR, 0:D] = full[lo:lo + GR]
            return pltpu.bitcast(wt[r][-8:, 3 * L:4 * L], I32)

        def repack(r):
            x = pltpu.bitcast(xb[r * 16:r * 16 + 16, :], I32)
            xbp[r * 8:r * 8 + 8, :] = x
            return functools.reduce(jnp.bitwise_and, [x[:, i:i + L] for i in range(0, S, L)])

        jobs = []
        nw, nx = pl.cdiv(3 * D, L), D // 16
        for r in range(nw):
            jobs.append(functools.partial(transpose, r))
            jobs += [functools.partial(repack, i)
                     for i in range(r * nx // nw, (r + 1) * nx // nw)]
        for g in range(G):
            kb[g * KROWS:g * KROWS + 48, 0:L] = jnp.zeros((48, L), I32)
        on_vpu = [[[] for _ in range(NT)] for _ in range(NCC)]
        later = []
        for cc in range(NCC):
            n = (cc + 1) * VPU_FIRST // NCC - cc * VPU_FIRST // NCC
            for k in range(n):
                t = len(later) % NT
                g = min(g for g in range(8)
                        if cc % NCH * 8 + g in vpu_slot and g not in on_vpu[cc][t])
                on_vpu[cc][t].append(g)
                later.append((cc, t, g, "k", cc, (2 * k + 1) * 7 // n))
        arrived(3)
        scores = []
        after = []
        for j in range(U):
            q = [q_tile(j, t).astype(BF) for t in range(NT)]
            for cc in range(j * NCH, (j + 1) * NCH):
                scores.append(make_probs(
                    j, q, cc, on_vpu[cc], [x[1:3] for x in later if x[0] == cc], after))
                todo = jobs[cc * len(jobs) // (NCC - 1):(cc + 1) * len(jobs) // (NCC - 1)]
                after = [((cc + i) % NT, job()) for i, job in enumerate(todo)]
        make_later_probs(0, later, scores, None)

    def middle_units(i, bad):
        steps = project_b_steps(i)
        loaded = {}
        scores = []
        for j in range(U):
            u = i * U + j
            q = [q_tile(u + U, t).astype(BF) for t in range(NT)]
            acc = [None] * NT
            for cc in range(j * NCH, (j + 1) * NCH):
                use_probs(cc, acc, loaded)
                loaded = {(t, g): p_a[p_tile(cc + 1, g, t)] for _, t, g in tied.get(cc, [])}
                qc = list(q)
                for k, t, g in tied.get(cc, []):
                    w = q_tile(u + U, t)
                    none = loaded[t, g] & pltpu.bitcast(zero(), I32)
                    qc[t] = jnp.concatenate(
                        [pltpu.bitcast(pltpu.bitcast(w[r:r + 8], I32) | none, F32)
                         if r == k * 16 else w[r:r + 8] for r in range(0, 32, 8)],
                        axis=0).astype(BF)
                scores.append(make_probs(
                    u + U, qc, cc, pos[cc], [x[1:3] for x in follow if x[0] == cc]))
            if j == U - 1:
                steps = [step() for step in steps]
            bad = finish(u, j, acc, bad)
        make_later_probs((i + 1) * U, follow, scores, steps)
        return bad

    first_units()
    bad = lax.fori_loop(0, UNITS // U - 1, middle_units, jnp.zeros((8, L), F32))

    def lane(rows):
        return lax.broadcasted_iota(I32, (rows, L), 1)

    def row(rows):
        return lax.broadcasted_iota(I32, (rows, L), 0)

    for u in range(4):
        lo = (((lane(40) >> 5) + u) & 3) * (DH // 2)
        qmask[u] = jnp.where((row(40) >= lo) & (row(40) < lo + DH // 2), -1, 0)

    def first_block(t):
        return max(0, 5 - 4 * t) if isinstance(t, int) else 0

    def scores_b(g, t):
        l16 = lane(16)
        slot = ((l16 >= DH).astype(I32) + (l16 >= 2 * DH).astype(I32)
                + (l16 >= 3 * DH).astype(I32))
        odd = (slot & 1) == 1
        q = qb[pl.ds(pl.multiple_of(g * 40, 8), 40), pl.ds(t * L, L)]
        qs = [pltpu.bitcast(_pad_rows(q & qmask[u], L // 2), BF) for u in range(4)]
        keys = {}
        half = {}

        def key(i):
            if i not in keys:
                start = pl.multiple_of(g * KROWS + (4 * t - 5 + i) * 16, 16)
                keys[i] = kb[pl.ds(start, 16), 0:L]
            return keys[i]

        def shifted(parity, i):
            if (parity, i) not in half:
                a, b = (key(i + 1), key(i)) if parity == 0 else (key(i), key(i + 1))
                half[parity, i] = jnp.where(odd, a, b)
            return half[parity, i]

        mx = [None] * 4

        def part(c):
            if c:
                return
            blocks = range(8, first_block(t) - 1, -1)
            for u in range(4):
                two = ((slot - u) & 2) == 2
                k = jnp.concatenate([jnp.where(two, shifted(u & 1, i + 2), shifted(u & 1, i))
                                     for i in blocks], axis=0)
                s = _dot(pltpu.bitcast(k, BF), qs[u])
                for n, i in enumerate(blocks):
                    si = s[32 * n:32 * n + 32]
                    if i == 0:
                        si = jnp.where((lane(32) & 31) < row(32), si, NEG)
                    elif i == 8:
                        si = jnp.where((lane(32) & 31) >= row(32), si, NEG)
                    elif i < 8 - 4 * t:
                        si = jnp.where((lane(32) >> 5) >= 8 - 4 * t - i, si, NEG)
                    s_b[pl.ds(t * 288 + 32 * i, 32), pl.ds(u * L, L)] = si
                    mc = jnp.max(si.reshape(4, 8, L), axis=0)
                    mx[u] = mc if mx[u] is None else jnp.maximum(mx[u], mc)

        def done():
            for u in range(4):
                m_b[pl.ds(t * 8, 8), pl.ds(u * L, L)] = jnp.broadcast_to(
                    jnp.max(mx[u], axis=0, keepdims=True), (8, L))

        return part, done

    def probs_b(t, slot=None):
        m = [m_b[_at(t * 8, 8), pl.ds(u * L, L)] for u in range(4)]
        dst, base = (p_b, t) if slot is None else (p_a, slot)

        def part(c):
            for i in ((0,), (4, 3, 2, 1), (8, 7, 6, 5))[c]:
                if i >= first_block(t):
                    for u in range(4):
                        s = s_b[_at(t * 288 + 32 * i, 32), pl.ds(u * L, L)]
                        p = jnp.exp2(s - jnp.concatenate([m[u]] * 4, axis=0)).astype(BF)
                        dst[_at(base * 144 + 16 * i, 16), pl.ds(u * L, L)] = (
                            pltpu.bitcast(p, I32))

        return part, lambda: None

    def values_b(g, t, out=None, slot=None):
        b0 = ((lane(16) >> 5) & 1) == 1
        b1 = ((lane(16) >> 5) & 2) == 2
        nothing = jnp.zeros((16, L), I32)
        src, base = (p_b, t) if slot is None else (p_a, slot)
        probs = {}
        half = {}

        def prob(u, i):
            if not first_block(t) <= i < 9:
                return nothing
            if (u, i) not in probs:
                probs[u, i] = src[_at(base * 144 + 16 * i, 16), pl.ds(u * L, L)]
            return probs[u, i]

        def shifted(u, i):
            if not first_block(t) <= i < 10:
                return nothing
            if (u, i) not in half:
                half[u, i] = jnp.where(b0, prob((u - 1) % 4, i - 1), prob(u, i))
            return half[u, i]

        acc = [None] * 4

        def part(c):
            if isinstance(t, int) and t - 2 + c < 0:
                return
            for j in range(4):
                p = jnp.concatenate(
                    [jnp.where(b1, shifted((j - 2) % 4, i - 2), shifted(j, i))
                     for i in range(4 * c, 4 * c + 4)], axis=0)
                v = [vb[g, pl.ds(16 * j + 8 * i, 8), _at((t - 2 + c) * L, L)] for i in range(3)]
                r = ONES_ROW[j]
                v[r // 8] = jnp.where(row8 == r % 8, 1.0, v[r // 8])
                o = _dot(jnp.concatenate(v, axis=0), pltpu.bitcast(p, BF))
                acc[j] = o + (kat[:, pl.ds(j * L, L)] if acc[j] is None else acc[j])

        def done():
            o = _join_heads([a * _recip24(a[r:r + 1]) for a, r in zip(acc, ONES_ROW)])
            if out is None:
                ob[g, :, _at(t * L, L)] = o
            else:
                ob2[out[0], :, pl.ds(out[1] * L, L)] = o

        return part, done

    def run(*stages):
        for c in (2, 1, 0):
            for part, _ in stages:
                part(c)
        for _, done in stages:
            done()

    steps = project_b_steps(UNITS // U - 1)
    for j in range(U):
        acc = [None] * NT
        for cc in range(j * NCH, (j + 1) * NCH):
            use_probs(cc, acc, {})
            if cc % 4 == 3 and cc // 4 < NSTEP:
                steps[cc // 4]()
            if cc % 4 == 1:
                run(scores_b(0, cc // 4))
        bad = finish(UNITS - U + j, j, acc, bad)

    @pl.when(jnp.max(bad) > 0.0)
    def _():
        def exact(u, carry):
            kbc[u, 0] = jnp.zeros((16, L), F32)
            q = _pad_rows(jnp.where(row24 == DH, 0.0, qa[u, 0:24]), 32).astype(BF)

            def scores(c, mx):
                k = pltpu.bitcast(ka[pl.ds(pl.multiple_of(c * 256, 256), 256), :], BF)
                s = _dot(k, q)
                p_a[pl.ds(pl.multiple_of(c * 512, 512), 512), :] = pltpu.bitcast(s, I32)
                return jnp.maximum(mx, jnp.max(s, axis=0, keepdims=True))

            m = lax.fori_loop(0, S // 512, scores, jnp.full((1, NB), -jnp.inf, F32))

            def values(c, acc):
                keys = pl.ds(pl.multiple_of(c * 512, 512), 512)
                p = jnp.exp2(pltpu.bitcast(p_a[keys, :], F32) - m).astype(BF)
                return acc + _dot(va[pl.ds(pl.multiple_of((u & 3) * 32, 32), 24), keys], p)

            oa[u] = lax.fori_loop(0, S // 512, values, jnp.zeros((24, NB), F32))
            return carry

        lax.fori_loop(0, UNITS, exact, 0)

    for t in range(NCH):
        run(probs_b(t), scores_b(1, t))

    def middle_groups(g, carry):
        for t in range(NCH):
            run(values_b(g, t), probs_b(t), scores_b(g + 2, t))
        return carry

    lax.fori_loop(0, G - 2, middle_groups, 0)

    arrived(4)

    def last_groups(n, buf):
        jobs = []
        for i in range(2):
            t, slot = 2 * n + i, 2 * buf + i
            jobs.append(lambda t=t, slot=slot: run(values_b(G - 2, t, (0, slot)),
                                                   probs_b(t, slot)))
            jobs.append(lambda t=t, slot=slot: run(values_b(G - 1, t, (1, slot), slot)))
        return jobs

    def out_block(n, buf, first=False, last=False):
        cols = _at(n * OUT_NB, OUT_NB)
        u0 = (n >> 1) * H
        sub = _at((n & 1) * OUT_NB, OUT_NB)
        heads_b = lambda: jnp.concatenate(
            [ob[g, :, cols] for g in range(G - 2)]
            + [ob2[g, :, pl.ds(buf * OUT_NB, OUT_NB)] for g in range(2)], axis=0).astype(BF)
        b = None if first else heads_b()
        a = jnp.concatenate(
            [_join_heads([oa[u0 + 4 * g + j, :, sub]
                          * _recip24(oa[u0 + 4 * g + j, pl.ds(ONES_ROW[j], 1), sub])
                          for j in range(4)]) for g in range(G)], axis=0).astype(BF)
        wt = wot
        if first:
            wt = jnp.concatenate([w[:, r:min(r + L, D)].T
                                  for w in (woa, wob) for r in range(0, D, L)], axis=0)
            wot[...] = wt
        side = (last_groups(n, buf) if first else []) + (
            [] if last else last_groups(n + 1, 1 - buf))
        tiles = range(2 * D // L)
        for i, j in enumerate(tiles if first else reversed(tiles)):
            for job in side[i:i + 1] if first else side[i // 2:i // 2 + i % 2]:
                job()
            r0, r1 = j * L, (j + 1) * L
            lhs = wt[r0:r1, :]
            res = []
            if r0 < D:
                res.append(_dot(lhs[0:min(r1, D) - r0], a))
            if r1 > D:
                b = heads_b() if b is None else b
                res.append(_dot(lhs[max(r0, D) - r0:L], b))
            obuf[cols, r0:r1] = jnp.concatenate(res, axis=0).T.astype(BF)

    def out_copy(i, n, count):
        rows = _at(n * OUT_NB, count * OUT_NB)
        return pltpu.make_async_copy(obuf.at[rows], out_hbm.at[rows], out_sem.at[i])

    nout = S // OUT_NB
    nmid = nout // 2 - 1
    out_block(0, 1, first=True)
    out_copy(nmid, 0, 1).start()

    def middle_blocks(i, carry):
        out_block(1 + 2 * i, 0)
        out_block(2 + 2 * i, 1)
        out_copy(i, 1 + 2 * i, 2).start()
        return carry

    lax.fori_loop(0, nmid, middle_blocks, 0)
    out_block(nout - 1, 0, last=True)
    out_copy(nmid + 1, nout - 1, 1).start()
    out_copy(nmid, 0, 1).wait()
    for i in range(nmid):
        out_copy(i, 1 + 2 * i, 2).wait()
    out_copy(nmid + 1, nout - 1, 1).wait()


@jax.jit
def pallas_concat_heads__grouped_kv_mqa__sliding_block__prompt_kernel(
    A_x: jax.Array,
    A_wq: jax.Array,
    A_wk: jax.Array,
    A_wv: jax.Array,
    A_wo: jax.Array,
    B_x: jax.Array,
    B_wqkv: jax.Array,
    B_wo: jax.Array,
):
    hbm = pl.BlockSpec(memory_space=pltpu.HBM)
    vmem = pltpu.VMEM
    scratch = [
        vmem((D, S), BF), vmem((D, S), BF),
        vmem((D, D), BF), vmem((D, D), BF),
        vmem((D, 3 * D), BF), vmem((D, D), BF),
        vmem((D, D), BF), vmem((G, 256, 5 * L), F32),
        vmem((2 * D, D), BF), vmem((D // 2, S), I32),
        vmem((UNITS, 32, NB), F32), vmem((24, S), F32),
        vmem((S // 2, 32), I32), vmem((UNITS, DH, 16, L), F32),
        vmem((128, S), F32), vmem((U * S // 2, NB), I32),
        vmem((UNITS, 24, NB), F32),
        vmem((G * 40, S), I32), vmem((G * KROWS, 2 * L), I32),
        vmem((G, GR, S), F32), vmem((NCH * 288, NB), F32),
        vmem((NCH * 144, NB), I32), vmem((NCH * 8, NB), F32),
        vmem((G - 2, GR, S), F32), vmem((2, GR, 2 * OUT_NB), F32),
        vmem((4, 40, L), I32), vmem((S, 2 * D), BF),
        vmem((DH, D), BF), vmem((DH, D), BF),
        pltpu.SemaphoreType.DMA((12,)), pltpu.SemaphoreType.DMA((S // OUT_NB // 2 + 1,)),
    ]
    out = pl.pallas_call(
        _kernel,
        in_specs=[hbm] * 8,
        out_specs=hbm,
        out_shape=jax.ShapeDtypeStruct((S, 2 * D), BF),
        scratch_shapes=scratch,
        compiler_params=pltpu.CompilerParams(vmem_limit_bytes=110 * 2**20),
        name="fused_attention",
    )(A_x.reshape(S, D).T, A_wq, A_wk.T, A_wv.T, A_wo, B_x.reshape(S, D).T, B_wqkv, B_wo)
    return out.reshape(1, S, 2 * D)
```
